```python
import jax
import jax.numpy as jnp

def _softmax(x, axis=-1):
    return jax.nn.softmax(x, axis=axis)
def _gelu(x):
    return jax.nn.gelu(x, approximate=True)
def _silu(x):
    return jax.nn.silu(x)
def _sigmoid(x):
    return jax.nn.sigmoid(x)
def _layernorm(x, axis=-1, eps=1e-5):
    m = jnp.mean(x, axis=axis, keepdims=True)
    v = jnp.var(x, axis=axis, keepdims=True)
    return (x - m) / jnp.sqrt(v + eps)
def _scatter_add(tgt, idx, src, axis=0):
    return tgt.at[idx].add(src)
def _segment_sum(src, seg, n):
    return jax.ops.segment_sum(src, seg, n)
class _Rng:
    def __init__(self, key):
        self._k = key
    def _next(self):
        self._k, sub = jax.random.split(self._k)
        return sub
    def normal(self, shape):
        return jax.random.normal(self._next(), shape, dtype=jnp.bfloat16)
    def randint(self, lo, hi, shape):
        return jax.random.randint(self._next(), shape, lo, hi, dtype=jnp.int32)
    def uniform(self, shape, lo=0.0, hi=1.0):
        return jax.random.uniform(self._next(), shape, jnp.bfloat16, lo, hi)
    def permutation(self, n):
        return jax.random.permutation(self._next(), n)


kernel_name = 'recurrent_scan__sliding_block_cached__mixer_s_mlp__decode'

def setup_inputs():
    _rng = _Rng(jax.random.key(int.from_bytes(__import__("os").urandom(4), "little")))
    _w = (lambda a: (lambda t: t.astype(jnp.bfloat16) if jnp.issubdtype(t.dtype, jnp.floating) else t)(jnp.asarray(a)))
    def _A_setup():
        B, Sq, D = 1, 1, 512
        Hq, Hkv, Sk, Dh = 32, 32, 32768, 128
        assert Hq % Hkv == 0, (Hq, Hkv)
        return {
            "x": _w((lambda *s: _rng.normal(s) * 0.05)(B, Sq, D)),
            "k_cache": _w((lambda *s: _rng.normal(s) * 0.05)(B, Hkv, Sk, Dh)),
            "v_cache": _w((lambda *s: _rng.normal(s) * 0.05)(B, Hkv, Sk, Dh)),
            "wq": _w((lambda *s: _rng.normal(s) * 0.05)(D, Hq * Dh) * (D ** -0.5)),
            "wo": _w((lambda *s: _rng.normal(s) * 0.05)(Hq * Dh, D) * ((Hq * Dh) ** -0.5)),
        }
    _A_in = _A_setup()

    def _B_setup():
        B, S, D, F = 1, 1, 512, 1376
        return {
            "x":  _w((lambda *s: _rng.normal(s) * 0.05)(B, S, D)),
            "w1": _w((lambda *s: _rng.normal(s) * 0.05)(D, D) * (D ** -0.5)),
            "w2": _w((lambda *s: _rng.normal(s) * 0.05)(D, D) * (D ** -0.5)),
            "w3": _w((lambda *s: _rng.normal(s) * 0.05)(D, F) * (D ** -0.5)),
            "w4": _w((lambda *s: _rng.normal(s) * 0.05)(F, D) * (F ** -0.5)),
        }
    _B_in = _B_setup()

    return {
        "A_x": _A_in["x"],
        "A_k_cache": _A_in["k_cache"],
        "A_v_cache": _A_in["v_cache"],
        "A_wq": _A_in["wq"],
        "A_wo": _A_in["wo"],
        "B_x": _B_in["x"],
        "B_w1": _B_in["w1"],
        "B_w2": _B_in["w2"],
        "B_w3": _B_in["w3"],
        "B_w4": _B_in["w4"],
    }

def reference(A_x, A_k_cache, A_v_cache, A_wq, A_wo, B_x, B_w1, B_w2, B_w3, B_w4):
    def _A_ref(x, k_cache, v_cache, wq, wo):
        B, Sq, D = x.shape
        Hq, Dh = 32, 128
        Hkv, Sk = k_cache.shape[1], k_cache.shape[2]
        W = min(4096, max(256, Sk // 4))
        rep = Hq // Hkv
        q = (lambda x, *d: x.transpose(*d))((x @ wq).reshape(B, Sq, Hq, Dh), 0, 2, 1, 3)
        k = jnp.repeat(k_cache[:, :, Sk - W:, :], rep, axis=1)
        v = jnp.repeat(v_cache[:, :, Sk - W:, :], rep, axis=1)
        scores = jnp.einsum("bhqd,bhkd->bhqk", q, k) * (Dh ** -0.5)
        p = _softmax(scores, axis=-1)
        o = jnp.einsum("bhqk,bhkd->bhqd", p, v)
        return (lambda x, *d: x.transpose(*d))(o, 0, 2, 1, 3).reshape(B, Sq, Hq * Dh) @ wo

    def _B_ref(x, w1, w2, w3, w4):
        B, S, D = x.shape
        h = _gelu(_layernorm(x, axis=-1) @ w1)
        c = D // 4
        g0 = jnp.pad(h[:, :, 0*c:1*c], ((0, 0), (1, 0), (0, 0)))[:, :S, :]
        g1 = jnp.pad(h[:, :, 1*c:2*c], ((0, 0), (0, 1), (0, 0)))[:, 1:, :]
        g2 = jnp.pad(h[:, :, 2*c:3*c], ((0, 0), (2, 0), (0, 0)))[:, :S, :]
        g3 = jnp.pad(h[:, :, 3*c:   ], ((0, 0), (0, 2), (0, 0)))[:, 2:, :]
        hs = jnp.concatenate([g0, g1, g2, g3], axis=-1) @ w2
        x1 = x + hs
        h2 = _gelu(_layernorm(x1, axis=-1) @ w3) @ w4
        return x1 + h2

    x = A_x
    xn = _layernorm(x, axis=-1)
    s = _A_ref(xn, A_k_cache, A_v_cache, A_wq, A_wo)
    g = _silu(_B_ref(xn, B_w1, B_w2, B_w3, B_w4))
    return x + s * g
```

```python
import functools
import jax
import jax.numpy as jnp
import numpy as np
import jax.experimental.pallas as pl
import jax.experimental.pallas.tpu as pltpu

D = 512
H = 32
DH = 128
F = 1376


def _ln(x):
    m = jnp.mean(x, axis=-1, keepdims=True)
    c = x - m
    v = jnp.mean(c * c, axis=-1, keepdims=True)
    return c / jnp.sqrt(v + 1e-5)


def build(look=3, vch=1024, nowait=False):
    def f(A_x, A_k_cache, A_v_cache, A_wq, A_wo, B_x, B_w1, B_w2, B_w3, B_w4):
        SK = A_k_cache.shape[2]
        W = min(4096, max(256, SK // 4))
        NV = W // vch

        def kern(x_hbm, k_hbm, v_hbm, wq_hbm, wo_hbm, w3_hbm, w4_hbm, o_ref,
                 xb, kb, vb, wqb, wob, w3b, w4b, qb, ksem, vsem, osem, msem):
            def k_cp(h):
                return pltpu.make_async_copy(k_hbm.at[0, h, pl.ds(SK - W, W), :], kb.at[h], ksem.at[h])
            def v_cp(h, c):
                return pltpu.make_async_copy(v_hbm.at[0, h, pl.ds(SK - W + c * vch, vch), :],
                                             vb.at[h, pl.ds(c * vch, vch), :], vsem.at[h * NV + c])
            def o_cp(h):
                r = pl.multiple_of(h * DH, DH)
                return pltpu.make_async_copy(wo_hbm.at[pl.ds(r, DH), :], wob.at[pl.ds(r, DH), :], osem.at[h])
            def start_head(h):
                k_cp(h).start()
                o_cp(h).start()
                for c in range(NV):
                    v_cp(h, c).start()
            wq_cp = pltpu.make_async_copy(wq_hbm, wqb, msem.at[0])
            x_cp = pltpu.make_async_copy(x_hbm, xb, msem.at[1])
            w3_cp = pltpu.make_async_copy(w3_hbm, w3b, msem.at[2])
            w4_cp = pltpu.make_async_copy(w4_hbm, w4b, msem.at[3])
            x_cp.start()
            wq_cp.start()
            w3_cp.start()
            w4_cp.start()
            for h in range(look):
                start_head(h)
            x_cp.wait()
            x = xb[0].astype(jnp.float32)
            x8 = jnp.broadcast_to(x, (8, D))
            xn = _ln(x8).astype(jnp.bfloat16)
            xnf = xn.astype(jnp.float32)
            xn2 = _ln(xnf).astype(jnp.bfloat16)
            wq_cp.wait()
            q = jnp.dot(xn, wqb[...], preferred_element_type=jnp.float32)
            for h in range(H):
                qb[h] = q[:, h * DH:(h + 1) * DH]
            w3_cp.wait()
            t = jax.lax.dot_general(xn2, w3b[...], (((1,), (1,)), ((), ())), preferred_element_type=jnp.float32)
            t = jax.nn.gelu(t, approximate=True).astype(jnp.bfloat16)
            w4_cp.wait()
            h2 = jnp.dot(t, w4b[...], preferred_element_type=jnp.float32)
            g = jax.nn.silu(xnf + h2)

            def body(h, acc):
                @pl.when(h + look < H)
                def _():
                    start_head(h + look)
                qh = qb[h].astype(jnp.bfloat16)
                k_cp(h).wait()
                s = jax.lax.dot_general(qh, kb[h], (((1,), (1,)), ((), ())),
                                        preferred_element_type=jnp.float32) * (DH ** -0.5)
                m = jnp.max(s, axis=-1, keepdims=True)
                p = jnp.exp(s - m)
                l = jnp.sum(p, axis=-1, keepdims=True)
                pb = p.astype(jnp.bfloat16)
                o = jnp.zeros((8, DH), jnp.float32)
                for c in range(NV):
                    v_cp(h, c).wait()
                    o = o + jnp.dot(pb[:, c * vch:(c + 1) * vch], vb[h, pl.ds(c * vch, vch), :],
                                    preferred_element_type=jnp.float32)
                o = (o / l).astype(jnp.bfloat16)
                o_cp(h).wait()
                r = pl.multiple_of(h * DH, DH)
                return acc + jnp.dot(o, wob[pl.ds(r, DH), :], preferred_element_type=jnp.float32)

            s = jax.lax.fori_loop(0, H, body, jnp.zeros((8, D), jnp.float32))
            out = x8 + s * g
            o_ref[0] = out[0:1].astype(o_ref.dtype)

        any_spec = pl.BlockSpec(memory_space=pl.ANY)
        bf = jnp.bfloat16
        return pl.pallas_call(
            kern,
            out_shape=jax.ShapeDtypeStruct((1, 1, D), A_x.dtype),
            in_specs=[any_spec] * 7,
            scratch_shapes=[
                pltpu.VMEM((1, 1, D), bf),
                pltpu.VMEM((H, W, DH), bf),
                pltpu.VMEM((H, W, DH), bf),
                pltpu.VMEM((D, H * DH), bf),
                pltpu.VMEM((H * DH, D), bf),
                pltpu.VMEM((F, D), bf),
                pltpu.VMEM((F, D), bf),
                pltpu.VMEM((H, 8, DH), jnp.float32),
                pltpu.SemaphoreType.DMA((H,)),
                pltpu.SemaphoreType.DMA((H * NV,)),
                pltpu.SemaphoreType.DMA((H,)),
                pltpu.SemaphoreType.DMA((4,)),
            ],
            compiler_params=pltpu.CompilerParams(vmem_limit_bytes=100 * 1024 * 1024),
        )(A_x, A_k_cache, A_v_cache, A_wq, A_wo, B_w3.T, B_w4)
    return f


_impl = build(look=2, vch=4096)


@jax.jit
def pallas_recurrent_scan__sliding_block_cached__mixer_s_mlp__decode_kernel(
    A_x, A_k_cache, A_v_cache, A_wq, A_wo, B_x, B_w1, B_w2, B_w3, B_w4,
):
    return _impl(A_x, A_k_cache, A_v_cache, A_wq, A_wo, B_x, B_w1, B_w2, B_w3, B_w4)
```

```python
import jax
import jax.numpy as jnp
import numpy as np
import jax.experimental.pallas as pl
import jax.experimental.pallas.tpu as pltpu

DH = 128
G = 8
KT = 128
NB = 16
_NT = (((1,), (1,)), ((), ()))
_F32_MIN = float(np.finfo(np.float32).min)


def _ln(x):
    m = jnp.mean(x, axis=-1, keepdims=True)
    c = x - m
    v = jnp.mean(c * c, axis=-1, keepdims=True)
    return c / jnp.sqrt(v + 1e-5)


def build(L=6, unroll=1, dbc=True):
    def f(A_x, A_k_cache, A_v_cache, A_wq, A_wo, B_x, B_w1, B_w2, B_w3, B_w4):
        D = A_x.shape[-1]
        H, SK = A_k_cache.shape[1], A_k_cache.shape[2]
        F = B_w4.shape[0]
        W = min(4096, max(256, SK // 4))
        NJ = W // KT
        NS = (H // G) * NJ
        NQ = H // 4
        NM, FR = F // 256, F % 256
        NSEM = L + 1
        bf, f32 = jnp.bfloat16, jnp.float32

        def kern(x_hbm, k_hbm, v_hbm, wq_hbm, wo_hbm, w3_hbm, w4_hbm, o_ref,
                 xb, kvb, wqb, wob, mb, mrb, qb, ob, sems, xsem):
            def wq_batch(b):
                return [(wq_hbm.at[pl.ds(32 * c, 32), pl.ds(512 * b, 512)],
                         wqb.at[b, pl.ds(32 * c, 32), :]) for c in range(D // 32)], wqb.at[b]

            def mlp_batch(b):
                dst, n = (mb.at[b], 256) if b < NM else (mrb, FR)
                cps = []
                for c in range(n // 32):
                    for t, src in enumerate((w3_hbm, w4_hbm)):
                        cps.append((src.at[pl.ds(256 * b + 32 * c, 32), :],
                                    dst.at[t, pl.ds(32 * c, 32), :]))
                return cps, dst

            def kv_batch(s):
                h0 = (s // NJ) * G
                r = SK - W + (s % NJ) * KT
                if not isinstance(s, int):
                    r = pl.multiple_of(r, KT)
                cps = []
                for hh in range(G):
                    for t, src in enumerate((k_hbm, v_hbm)):
                        cps.append((src.at[0, h0 + hh, pl.ds(r, KT), :], kvb.at[s, 2 * hh + t]))
                return cps, kvb.at[s]

            def wo_batch(b):
                rows = [128 * (c % 4) + 32 * (c // 4) for c in range(16)]
                return [(wo_hbm.at[pl.ds(512 * b + r, 32), :], wob.at[b, pl.ds(r, 32), :])
                        for r in rows], wob.at[b]

            P1 = NQ
            P2 = P1 + NM + (1 if FR else 0)
            P3 = P2 + NS
            P4 = P3 + NQ

            def batch(i):
                if i < P1:
                    return wq_batch(i)
                if i < P2:
                    return mlp_batch(i - P1)
                if i < P3:
                    return kv_batch(i - P2)
                return wo_batch(i - P3)

            def start(cps, i):
                for t, (s, d) in enumerate(cps):
                    pltpu.make_async_copy(s, d, sems.at[i % NSEM]).start(priority=t % 2)

            def wait(buf, i):
                pltpu.make_async_copy(buf, buf, sems.at[i % NSEM]).wait()

            def advance(i):
                wait(batch(i)[1], i)
                if i + L < P4:
                    start(batch(i + L)[0], i + L)

            x_cp = pltpu.make_async_copy(x_hbm, xb, xsem.at[0])
            x_cp.start()
            for i in range(L):
                start(batch(i)[0], i)
            x_cp.wait()
            row = jax.lax.broadcasted_iota(jnp.int32, (G, DH), 0)
            x8 = jnp.broadcast_to(xb[0].astype(f32), (G, D))
            xn = _ln(x8).astype(bf)
            xnf = xn.astype(f32)
            xn2 = _ln(xnf).astype(bf)

            for b in range(NQ):
                advance(b)
                q = jnp.dot(xn, wqb[b], preferred_element_type=f32)
                for u in range(4):
                    h = 4 * b + u
                    qb[h] = jnp.where(row == h % G, q[:, u * DH:(u + 1) * DH], 0.0)

            h2 = jnp.zeros((G, D), f32)
            for b in range(P2 - P1):
                advance(P1 + b)
                w = mb.at[b] if b < NM else mrb
                t = jax.lax.dot_general(xn2, w[0], _NT, preferred_element_type=f32)
                t = jax.nn.gelu(t, approximate=True).astype(bf)
                h2 = h2 + jnp.dot(t, w[1], preferred_element_type=f32)
            gate = jax.nn.silu(xnf + h2)

            def attend(s, carry):
                m, l, acc = carry
                g = s // NJ
                first = (s % NJ) == 0
                m = jnp.where(first, _F32_MIN, m)
                l = jnp.where(first, 0.0, l)
                acc = jnp.where(first, 0.0, acc)
                sc = None
                for hh in range(G):
                    d = jax.lax.dot_general(qb[g * G + hh].astype(bf), kvb[s, 2 * hh], _NT,
                                            preferred_element_type=f32)
                    sc = d if sc is None else sc + d
                sc = sc * (DH ** -0.5)
                m_new = jnp.maximum(m, jnp.max(sc, axis=-1, keepdims=True))
                alpha = jnp.exp(m - m_new)
                p = jnp.exp(sc - m_new)
                l = alpha * l + p
                acc = alpha * acc
                for hh in range(G):
                    ph = jnp.where(row == hh, p, 0.0).astype(bf)
                    acc = acc + jnp.dot(ph, kvb[s, 2 * hh + 1], preferred_element_type=f32)
                ob[g, 0] = acc
                ob[g, 1] = l
                return m_new, l, acc

            def body(s, carry):
                wait(kvb.at[s], P2 + s)
                start(kv_batch(s + L)[0], P2 + s + L)
                return attend(s, carry)

            carry = (jnp.full((G, 1), _F32_MIN, f32), jnp.zeros((G, KT), f32), jnp.zeros((G, DH), f32))
            carry = jax.lax.fori_loop(0, NS - L, body, carry, unroll=unroll)
            for s in range(NS - L, NS):
                advance(P2 + s)
                carry = attend(s, carry)

            acc = jnp.zeros((G, D), f32)
            for b in range(NQ):
                g = (4 * b) // G
                o = ob[g, 0] / jnp.sum(ob[g, 1], axis=-1, keepdims=True)
                lhs = jnp.concatenate(
                    [jnp.where(row == (4 * b + u) % G, o, 0.0).astype(bf) for u in range(4)], axis=1)
                advance(P3 + b)
                acc = acc + jnp.dot(lhs, wob[b], preferred_element_type=f32)
            s_out = jnp.sum(acc, axis=0, keepdims=True)
            o_ref[0] = (x8[0:1] + s_out * gate[0:1]).astype(o_ref.dtype)

        any_spec = pl.BlockSpec(memory_space=pl.ANY)
        return pl.pallas_call(
            kern,
            out_shape=jax.ShapeDtypeStruct((1, 1, D), A_x.dtype),
            in_specs=[any_spec] * 7,
            scratch_shapes=[
                pltpu.VMEM((1, 1, D), bf),
                pltpu.VMEM((NS, 2 * G, KT, DH), bf),
                pltpu.VMEM((NQ, D, 512), bf),
                pltpu.VMEM((NQ, 512, D), bf),
                pltpu.VMEM((NM, 2, 256, D), bf),
                pltpu.VMEM((2, FR, D), bf),
                pltpu.VMEM((H, G, DH), f32),
                pltpu.VMEM((H // G, 2, G, DH), f32),
                pltpu.SemaphoreType.DMA((NSEM,)),
                pltpu.SemaphoreType.DMA((1,)),
            ],
            compiler_params=pltpu.CompilerParams(
                vmem_limit_bytes=100 * 1024 * 1024, disable_bounds_checks=dbc),
        )(A_x, A_k_cache, A_v_cache, A_wq, A_wo, B_w3.T, B_w4)
    return f


_impl = build(L=6)


@jax.jit
def pallas_recurrent_scan__sliding_block_cached__mixer_s_mlp__decode_kernel(
    A_x, A_k_cache, A_v_cache, A_wq, A_wo, B_x, B_w1, B_w2, B_w3, B_w4,
):
    return _impl(A_x, A_k_cache, A_v_cache, A_wq, A_wo, B_x, B_w1, B_w2, B_w3, B_w4)
```

```python
import jax
import jax.numpy as jnp
import numpy as np
import jax.experimental.pallas as pl
import jax.experimental.pallas.tpu as pltpu

DH = 128
G = 8
KT = 128
_NT = (((1,), (1,)), ((), ()))
_F32_MIN = float(np.finfo(np.float32).min)


def _ln(x):
    m = jnp.mean(x, axis=-1, keepdims=True)
    c = x - m
    v = jnp.mean(c * c, axis=-1, keepdims=True)
    return c / jnp.sqrt(v + 1e-5)


def build(L=6):
    def f(A_x, A_k_cache, A_v_cache, A_wq, A_wo, B_x, B_w1, B_w2, B_w3, B_w4):
        D = A_x.shape[-1]
        H, SK = A_k_cache.shape[1], A_k_cache.shape[2]
        F = B_w4.shape[0]
        W = min(4096, max(256, SK // 4))
        NJ = W // KT
        NS = (H // G) * NJ
        NQ = H // 4
        NM, FR = F // 256, F % 256
        NSEM = L + 1
        assert A_x.shape == (1, 1, 512) and A_k_cache.shape[3] == DH
        assert H % G == 0 and W % KT == 0 and SK % KT == 0 and NS > L and FR % 32 == 0
        bf, f32 = jnp.bfloat16, jnp.float32

        def kern(x_hbm, k_hbm, v_hbm, wq_hbm, wo_hbm, w3_hbm, w4_hbm, o_ref,
                 xb, kvb, wqb, wob, mb, mrb, qb, ob, sems, xsem):
            def wq_batch(b):
                return [(wq_hbm.at[pl.ds(32 * c, 32), pl.ds(512 * b, 512)],
                         wqb.at[b, pl.ds(32 * c, 32), :]) for c in range(D // 32)], wqb.at[b]

            def mlp_batch(b):
                dst, n = (mb.at[b], 256) if b < NM else (mrb, FR)
                cps = []
                for c in range(n // 32):
                    for t, src in enumerate((w3_hbm, w4_hbm)):
                        cps.append((src.at[pl.ds(256 * b + 32 * c, 32), :],
                                    dst.at[t, pl.ds(32 * c, 32), :]))
                return cps, dst

            def kv_batch(s):
                h0 = (s // NJ) * G
                r = SK - W + (s % NJ) * KT
                if not isinstance(s, int):
                    r = pl.multiple_of(r, KT)
                cps = []
                for hh in range(G):
                    for t, src in enumerate((k_hbm, v_hbm)):
                        cps.append((src.at[0, h0 + hh, pl.ds(r, KT), :], kvb.at[s, 2 * hh + t]))
                return cps, kvb.at[s]

            def wo_batch(b):
                rows = [128 * (c % 4) + 32 * (c // 4) for c in range(16)]
                return [(wo_hbm.at[pl.ds(512 * b + r, 32), :], wob.at[b, pl.ds(r, 32), :])
                        for r in rows], wob.at[b]

            P1 = NQ
            P2 = P1 + NM + (1 if FR else 0)
            P3 = P2 + NS
            P4 = P3 + NQ

            def batch(i):
                if i < P1:
                    return wq_batch(i)
                if i < P2:
                    return mlp_batch(i - P1)
                if i < P3:
                    return kv_batch(i - P2)
                return wo_batch(i - P3)

            def start(cps, i):
                for t, (s, d) in enumerate(cps):
                    pltpu.make_async_copy(s, d, sems.at[i % NSEM]).start(priority=t % 2)

            def wait(buf, i):
                pltpu.make_async_copy(buf, buf, sems.at[i % NSEM]).wait()

            def advance(i):
                wait(batch(i)[1], i)
                if i + L < P4:
                    start(batch(i + L)[0], i + L)

            x_cp = pltpu.make_async_copy(x_hbm, xb, xsem.at[0])
            x_cp.start()
            for i in range(L):
                start(batch(i)[0], i)
            x_cp.wait()
            row = jax.lax.broadcasted_iota(jnp.int32, (G, DH), 0)
            x8 = jnp.broadcast_to(xb[0].astype(f32), (G, D))
            xn = _ln(x8).astype(bf)
            xnf = xn.astype(f32)
            xn2 = _ln(xnf).astype(bf)

            for b in range(NQ):
                advance(b)
                q = jnp.dot(xn, wqb[b], preferred_element_type=f32)
                for u in range(4):
                    h = 4 * b + u
                    qb[h] = jnp.where(row == h % G, q[:, u * DH:(u + 1) * DH], 0.0)

            h2 = jnp.zeros((G, D), f32)
            for b in range(P2 - P1):
                advance(P1 + b)
                w = mb.at[b] if b < NM else mrb
                t = jax.lax.dot_general(xn2, w[0], _NT, preferred_element_type=f32)
                t = jax.nn.gelu(t, approximate=True).astype(bf)
                h2 = h2 + jnp.dot(t, w[1], preferred_element_type=f32)
            gate = jax.nn.silu(xnf + h2)

            def attend(s, carry):
                m, l, acc = carry
                g = s // NJ
                first = (s % NJ) == 0
                m = jnp.where(first, _F32_MIN, m)
                l = jnp.where(first, 0.0, l)
                acc = jnp.where(first, 0.0, acc)
                sc = None
                for hh in range(G):
                    d = jax.lax.dot_general(qb[g * G + hh].astype(bf), kvb[s, 2 * hh], _NT,
                                            preferred_element_type=f32)
                    sc = d if sc is None else sc + d
                sc = sc * (DH ** -0.5)
                m_new = jnp.maximum(m, jnp.max(sc, axis=-1, keepdims=True))
                alpha = jnp.exp(m - m_new)
                p = jnp.exp(sc - m_new)
                l = alpha * l + p
                acc = alpha * acc
                for hh in range(G):
                    ph = jnp.where(row == hh, p, 0.0).astype(bf)
                    acc = acc + jnp.dot(ph, kvb[s, 2 * hh + 1], preferred_element_type=f32)
                ob[g, 0] = acc
                ob[g, 1] = l
                return m_new, l, acc

            def body(s, carry):
                wait(kvb.at[s], P2 + s)
                start(kv_batch(s + L)[0], P2 + s + L)
                return attend(s, carry)

            carry = (jnp.full((G, 1), _F32_MIN, f32), jnp.zeros((G, KT), f32), jnp.zeros((G, DH), f32))
            carry = jax.lax.fori_loop(0, NS - L, body, carry)
            for s in range(NS - L, NS):
                advance(P2 + s)
                carry = attend(s, carry)

            acc = jnp.zeros((G, D), f32)
            for b in range(NQ):
                g = (4 * b) // G
                o = ob[g, 0] / jnp.sum(ob[g, 1], axis=-1, keepdims=True)
                lhs = jnp.concatenate(
                    [jnp.where(row == (4 * b + u) % G, o, 0.0).astype(bf) for u in range(4)], axis=1)
                advance(P3 + b)
                acc = acc + jnp.dot(lhs, wob[b], preferred_element_type=f32)
            s_out = jnp.sum(acc, axis=0, keepdims=True)
            o_ref[0] = (x8[0:1] + s_out * gate[0:1]).astype(o_ref.dtype)

        any_spec = pl.BlockSpec(memory_space=pl.ANY)
        return pl.pallas_call(
            kern,
            out_shape=jax.ShapeDtypeStruct((1, 1, D), A_x.dtype),
            in_specs=[any_spec] * 7,
            scratch_shapes=[
                pltpu.VMEM((1, 1, D), bf),
                pltpu.VMEM((NS, 2 * G, KT, DH), bf),
                pltpu.VMEM((NQ, D, 512), bf),
                pltpu.VMEM((NQ, 512, D), bf),
                pltpu.VMEM((NM, 2, 256, D), bf),
                pltpu.VMEM((2, FR, D), bf),
                pltpu.VMEM((H, G, DH), f32),
                pltpu.VMEM((H // G, 2, G, DH), f32),
                pltpu.SemaphoreType.DMA((NSEM,)),
                pltpu.SemaphoreType.DMA((1,)),
            ],
            compiler_params=pltpu.CompilerParams(vmem_limit_bytes=100 * 1024 * 1024),
        )(A_x, A_k_cache, A_v_cache, A_wq, A_wo, B_w3.T, B_w4)
    return f


_impl = build(L=6)


@jax.jit
def pallas_recurrent_scan__sliding_block_cached__mixer_s_mlp__decode_kernel(
    A_x, A_k_cache, A_v_cache, A_wq, A_wo, B_x, B_w1, B_w2, B_w3, B_w4,
):
    return _impl(A_x, A_k_cache, A_v_cache, A_wq, A_wo, B_x, B_w1, B_w2, B_w3, B_w4)
```
